```python
import os as _os
_os.environ.setdefault("JAX_PLATFORMS", "cpu")
import jax
import jax.numpy as jnp

def _softmax(x, axis=-1):
    return jax.nn.softmax(x, axis=axis)
def _gelu(x):
    return jax.nn.gelu(x, approximate=True)
def _silu(x):
    return jax.nn.silu(x)
def _sigmoid(x):
    return jax.nn.sigmoid(x)
def _layernorm(x, axis=-1, eps=1e-5):
    m = jnp.mean(x, axis=axis, keepdims=True)
    v = jnp.var(x, axis=axis, keepdims=True)
    return (x - m) / jnp.sqrt(v + eps)
def _scatter_add(tgt, idx, src, axis=0):
    return tgt.at[idx].add(src)
def _segment_sum(src, seg, n):
    return jax.ops.segment_sum(src, seg, n)
class _Rng:
    def __init__(self, key):
        self._k = key
    def _next(self):
        self._k, sub = jax.random.split(self._k)
        return sub
    def normal(self, shape):
        return jax.random.normal(self._next(), shape, dtype=jnp.bfloat16)
    def randint(self, lo, hi, shape):
        return jax.random.randint(self._next(), shape, lo, hi, dtype=jnp.int32)
    def uniform(self, shape, lo=0.0, hi=1.0):
        return jax.random.uniform(self._next(), shape, jnp.bfloat16, lo, hi)
    def permutation(self, n):
        return jax.random.permutation(self._next(), n)


kernel_name = 'concat_heads__gqa_block_cached__gqa_block_cached__near_ridge'

def setup_inputs():
    _rng = _Rng(jax.random.key(int.from_bytes(__import__("os").urandom(4), "little")))
    _w = (lambda a: (lambda t: t.astype(jnp.bfloat16) if jnp.issubdtype(t.dtype, jnp.floating) else t)(jnp.asarray(a)))
    def _A_setup():
        B, Sq, D = 8, 128, 576
        Hq, Hkv, Sk, Dh = 32, 16, 512, 128
        assert Hq % Hkv == 0, (Hq, Hkv)
        return {
            "x": _w((lambda *s: _rng.normal(s) * 0.8)(B, Sq, D)),
            "k_cache": _w((lambda *s: _rng.normal(s) * 0.8)(B, Hkv, Sk, Dh)),
            "v_cache": _w((lambda *s: _rng.normal(s) * 0.05)(B, Hkv, Sk, Dh)),
            "wq": _w((lambda *s: _rng.normal(s) * 0.8)(D, Hq * Dh) * (D ** -0.5)),
            "wo": _w((lambda *s: _rng.normal(s) * 0.05)(Hq * Dh, D) * ((Hq * Dh) ** -0.5)),
        }
    _A_in = _A_setup()

    def _B_setup():
        B, Sq, D = 8, 128, 576
        Hq, Hkv, Sk, Dh = 32, 16, 512, 128
        assert Hq % Hkv == 0, (Hq, Hkv)
        return {
            "x": _w((lambda *s: _rng.normal(s) * 0.8)(B, Sq, D)),
            "k_cache": _w((lambda *s: _rng.normal(s) * 0.8)(B, Hkv, Sk, Dh)),
            "v_cache": _w((lambda *s: _rng.normal(s) * 0.05)(B, Hkv, Sk, Dh)),
            "wq": _w((lambda *s: _rng.normal(s) * 0.8)(D, Hq * Dh) * (D ** -0.5)),
            "wo": _w((lambda *s: _rng.normal(s) * 0.05)(Hq * Dh, D) * ((Hq * Dh) ** -0.5)),
        }
    _B_in = _B_setup()

    return {
        "A_x": _A_in["x"],
        "A_k_cache": _A_in["k_cache"],
        "A_v_cache": _A_in["v_cache"],
        "A_wq": _A_in["wq"],
        "A_wo": _A_in["wo"],
        "B_x": _B_in["x"],
        "B_k_cache": _B_in["k_cache"],
        "B_v_cache": _B_in["v_cache"],
        "B_wq": _B_in["wq"],
        "B_wo": _B_in["wo"],
    }

def reference(A_x, A_k_cache, A_v_cache, A_wq, A_wo, B_x, B_k_cache, B_v_cache, B_wq, B_wo):
    def _A_ref(x, k_cache, v_cache, wq, wo):
        B, Sq, D = x.shape
        Hq, Dh = 32, 128
        Hkv = k_cache.shape[1]
        rep = Hq // Hkv
        q = (lambda x, *d: x.transpose(*d))((x @ wq).reshape(B, Sq, Hq, Dh), 0, 2, 1, 3)
        k = jnp.repeat(k_cache, rep, axis=1)
        v = jnp.repeat(v_cache, rep, axis=1)
        scores = jnp.einsum("bhqd,bhkd->bhqk", q, k) * (Dh ** -0.5)
        p = _softmax(scores, axis=-1)
        o = jnp.einsum("bhqk,bhkd->bhqd", p, v)
        return (lambda x, *d: x.transpose(*d))(o, 0, 2, 1, 3).reshape(B, Sq, Hq * Dh) @ wo

    def _B_ref(x, k_cache, v_cache, wq, wo):
        B, Sq, D = x.shape
        Hq, Dh = 32, 128
        Hkv = k_cache.shape[1]
        rep = Hq // Hkv
        q = (lambda x, *d: x.transpose(*d))((x @ wq).reshape(B, Sq, Hq, Dh), 0, 2, 1, 3)
        k = jnp.repeat(k_cache, rep, axis=1)
        v = jnp.repeat(v_cache, rep, axis=1)
        scores = jnp.einsum("bhqd,bhkd->bhqk", q, k) * (Dh ** -0.5)
        p = _softmax(scores, axis=-1)
        o = jnp.einsum("bhqk,bhkd->bhqd", p, v)
        return (lambda x, *d: x.transpose(*d))(o, 0, 2, 1, 3).reshape(B, Sq, Hq * Dh) @ wo

    a = _A_ref(A_x, A_k_cache, A_v_cache, A_wq, A_wo)
    b = _B_ref(B_x, B_k_cache, B_v_cache, B_wq, B_wo)
    return jnp.concatenate([a, b], axis=-1)
```

```python
import jax
import jax.numpy as jnp
from jax import lax
import jax.experimental.pallas as pl
import jax.experimental.pallas.tpu as pltpu

B, SQ, D = 8, 128, 576
HKV, SK, DH = 16, 512, 128
REP = 2
G = 2
NSTEP_B = HKV // G
NSTEP = 2 * NSTEP_B
HW = G * REP * DH
NS = 3
NT = (((1,), (1,)), ((), ()))
NN = (((1,), (0,)), ((), ()))
SCALE = float(DH ** -0.5 * 1.4426950408889634)
F32, BF16 = jnp.float32, jnp.bfloat16


def _region(name, f):
    del name
    f()


def kernel(xa, ka, va, wqa, woa, xb, kb, vb, wqb, wob, out_hbm,
           xt_buf, x_buf, k_buf, v_buf, wq_buf, wo_buf, q_buf, acc, ostage,
           sems, psem, osem):

    def cp_wq(wq_h, gg, slot):
        c0 = gg * HW if isinstance(gg, int) else pl.multiple_of(gg * HW, HW)
        return pltpu.make_async_copy(wq_h.at[:, pl.ds(c0, HW)], wq_buf.at[slot], sems.at[slot, 0])

    def cp_wo(wo_h, gg, slot):
        c0 = gg * HW if isinstance(gg, int) else pl.multiple_of(gg * HW, HW)
        return pltpu.make_async_copy(wo_h.at[:, pl.ds(c0, HW)], wo_buf.at[slot], sems.at[slot, 3])

    def cp_k(k_h, gg, slot):
        return pltpu.make_async_copy(k_h.at[:, pl.ds(gg * G, G)], k_buf.at[slot], sems.at[slot, 1])

    def cp_v(v_h, gg, slot):
        return pltpu.make_async_copy(v_h.at[:, pl.ds(gg * G, G)], v_buf.at[slot], sems.at[slot, 2])

    def start_step(i, slot):
        def go(k_h, v_h, wq_h, wo_h, gg):
            cp_wq(wq_h, gg, slot).start()
            cp_k(k_h, gg, slot).start()
            cp_v(v_h, gg, slot).start()
            cp_wo(wo_h, gg, slot).start()
        if isinstance(i, int):
            if i < NSTEP_B:
                go(ka, va, wqa, woa, i)
            elif i < NSTEP:
                go(kb, vb, wqb, wob, i - NSTEP_B)
        else:
            @pl.when(i < NSTEP_B)
            def _():
                go(ka, va, wqa, woa, i)

            @pl.when(jnp.logical_and(i >= NSTEP_B, i < NSTEP))
            def _():
                go(kb, vb, wqb, wob, i - NSTEP_B)

    def wait_step(slot):
        cp_wq(wqa, 0, slot).wait()
        cp_k(ka, 0, slot).wait()
        cp_v(va, 0, slot).wait()
        cp_wo(woa, 0, slot).wait()

    def cp_x(x_h, s, b0, nb, sem):
        return pltpu.make_async_copy(x_h.at[pl.ds(b0, nb)], xt_buf.at[s, pl.ds(b0, nb)], psem.at[sem])

    def cp_kv0(b0, nb, sem):
        return (pltpu.make_async_copy(ka.at[pl.ds(b0, nb), pl.ds(0, G)], k_buf.at[0, pl.ds(b0, nb)], psem.at[sem]),
                pltpu.make_async_copy(va.at[pl.ds(b0, nb), pl.ds(0, G)], v_buf.at[0, pl.ds(b0, nb)], psem.at[sem + 1]))

    def xpose_x(s, b):
        x_buf[s, pl.ds(b * SQ, SQ), :] = xt_buf[s, b].T

    def run_step(slot, s, order, hooks):
        r0 = s * D if isinstance(s, int) else pl.multiple_of(s * D, 8)
        svals, ovals = {}, {}

        def jobQ(b):
            x = x_buf[s, pl.ds(b * SQ, SQ), :]
            q = lax.dot_general(x, wq_buf[slot], NN, preferred_element_type=F32)
            q = (q * SCALE).astype(BF16)
            for h in range(G * REP):
                q_buf[h // REP, b, pl.ds((h % REP) * SQ, SQ), :] = q[:, h * DH:(h + 1) * DH]

        def jobS(b):
            for j in range(G):
                sc = lax.dot_general(q_buf[j, b], k_buf[slot, b, j], NT, preferred_element_type=F32)
                m = jnp.max(sc, axis=-1, keepdims=True)
                p = jnp.exp2(sc - m)
                l = jnp.sum(p, axis=-1, keepdims=True)
                svals[b, j] = (p.astype(BF16), l)

        def jobP(b):
            for j in range(G):
                p, l = svals.pop((b, j))
                o = lax.dot_general(p, v_buf[slot, b, j], NN, preferred_element_type=F32)
                inv = pltpu.reciprocal(l, approx=True)
                inv = inv * (2.0 - l * inv)
                ovals[b, j] = (o * inv).astype(BF16)

        def jobO(b):
            parts = []
            for j in range(G):
                o = ovals.pop((b, j))
                parts += [o[:SQ], o[SQ:]]
            ob = jnp.concatenate(parts, axis=1)
            r = lax.dot_general(wo_buf[slot], ob, NT, preferred_element_type=F32)
            acc[pl.ds(r0, D), pl.ds(b * SQ, SQ)] += r

        jobs = dict(Q=jobQ, S=jobS, P=jobP, O=jobO)
        for name in order:
            if name in hooks:
                hooks[name]()
            jobs[name[0]](int(name[1:]))

    order = [f"Q{b}" for b in range(B)]
    for b in range(B):
        order += [f"S{b}", f"P{b}"]
    order += [f"O{b}" for b in range(B)]

    x01 = cp_x(xa, 0, 0, 2, 0)
    x27 = cp_x(xa, 0, 2, 6, 1)
    kva = cp_kv0(0, 4, 2)
    kvb = cp_kv0(4, 4, 4)
    xbc = cp_x(xb, 1, 0, B, 6)

    def p0():
        cp_wq(wqa, 0, 0).start()
        x01.start()
        x27.start()
        acc[...] = jnp.zeros(acc.shape, F32)

    _region("p0", p0)

    def h_q0():
        cp_wq(wqa, 0, 0).wait()
        x01.wait()
        kva[0].start(); kva[1].start()
        xpose_x(0, 0); xpose_x(0, 1)

    def h_q2():
        x27.wait()
        kvb[0].start(); kvb[1].start()
        for b in range(2, B):
            xpose_x(0, b)

    def h_s0():
        kva[0].wait(); kva[1].wait()
        cp_wo(woa, 0, 0).start()
        cp_wq(wqa, 1, 1).start()

    def h_s4():
        kvb[0].wait(); kvb[1].wait()
        cp_k(ka, 1, 1).start(); cp_v(va, 1, 1).start(); cp_wo(woa, 1, 1).start()

    def h_o0():
        cp_wo(woa, 0, 0).wait()
        cp_wq(wqa, 1, 1).wait()
        start_step(2, 2)

    _region("s0", lambda: run_step(0, 0, order, {"Q0": h_q0, "Q2": h_q2, "S0": h_s0, "S4": h_s4, "O0": h_o0}))

    def h1_s0():
        cp_k(ka, 1, 1).wait(); cp_v(va, 1, 1).wait(); cp_wo(woa, 1, 1).wait()
        xbc.start()

    def h1_s4():
        start_step(3, 0)

    _region("s1", lambda: run_step(1, 0, order, {"S0": h1_s0, "S4": h1_s4}))

    def body(i, carry):
        slot = lax.rem(i, NS)
        s = i // NSTEP_B

        @pl.when(i == NSTEP_B)
        def _():
            xbc.wait()
            for b in range(B):
                xpose_x(1, b)
            for b in range(B):
                ostage[b, :, 0:512] = acc[0:512, pl.ds(b * SQ, SQ)].T.astype(BF16)
            pltpu.make_async_copy(ostage.at[:, :, pl.ds(0, 512)], out_hbm.at[:, :, pl.ds(0, 512)], osem.at[B]).start()

        wait_step(slot)
        run_step(slot, s, order, {"Q4": lambda: start_step(i + 2, lax.rem(i + 2, NS))})
        return carry

    _region("loop", lambda: lax.fori_loop(2, NSTEP, body, 0))

    def epi():
        for b in range(B):
            ostage[b, :, 512:1152] = acc[512:1152, pl.ds(b * SQ, SQ)].T.astype(BF16)
            pltpu.make_async_copy(ostage.at[b, :, pl.ds(512, 640)], out_hbm.at[b, :, pl.ds(512, 640)], osem.at[b]).start()
        pltpu.make_async_copy(ostage.at[:, :, pl.ds(0, 512)], out_hbm.at[:, :, pl.ds(0, 512)], osem.at[B]).wait()
        for b in range(B):
            pltpu.make_async_copy(ostage.at[b, :, pl.ds(512, 640)], out_hbm.at[b, :, pl.ds(512, 640)], osem.at[b]).wait()

    _region("epi", epi)


@jax.jit
def pallas_concat_heads__gqa_block_cached__gqa_block_cached__near_ridge_kernel(A_x, A_k_cache, A_v_cache, A_wq, A_wo, B_x, B_k_cache, B_v_cache, B_wq, B_wo):
    hbm = pl.BlockSpec(memory_space=pltpu.HBM)
    out = pl.pallas_call(
        kernel,
        grid=(1,),
        in_specs=[hbm] * 10,
        out_specs=hbm,
        out_shape=jax.ShapeDtypeStruct((B, SQ, 2 * D), BF16),
        scratch_shapes=[
            pltpu.VMEM((2, B, D, SQ), BF16),
            pltpu.VMEM((2, B * SQ, D), BF16),
            pltpu.VMEM((NS, B, G, SK, DH), BF16),
            pltpu.VMEM((NS, B, G, SK, DH), BF16),
            pltpu.VMEM((NS, D, HW), BF16),
            pltpu.VMEM((NS, D, HW), BF16),
            pltpu.VMEM((G, B, REP * SQ, DH), BF16),
            pltpu.VMEM((2 * D, B * SQ), F32),
            pltpu.VMEM((B, SQ, 2 * D), BF16),
            pltpu.SemaphoreType.DMA((NS, 4)),
            pltpu.SemaphoreType.DMA((8,)),
            pltpu.SemaphoreType.DMA((B + 1,)),
        ],
        compiler_params=pltpu.CompilerParams(vmem_limit_bytes=100 * 1024 * 1024, disable_bounds_checks=True),
    )(A_x.transpose(0, 2, 1), A_k_cache, A_v_cache, A_wq, A_wo.T,
      B_x.transpose(0, 2, 1), B_k_cache, B_v_cache, B_wq, B_wo.T)
    return out
```

```python
import jax
import jax.numpy as jnp
from jax import lax
import jax.experimental.pallas as pl
import jax.experimental.pallas.tpu as pltpu

B, SQ, D = 8, 128, 576
HKV, SK, DH = 16, 512, 128
REP = 2
G = 2
NSTEP_B = HKV // G
NSTEP = 2 * NSTEP_B
HW = G * REP * DH
NS = 3
NT = (((1,), (1,)), ((), ()))
NN = (((1,), (0,)), ((), ()))
SCALE = float(DH ** -0.5 * 1.4426950408889634)
F32, BF16 = jnp.float32, jnp.bfloat16

KSPLIT = 6
ORD = "QF"
HK1 = "Q1"
HK2 = "S2"


def _bind(f, *a):
    return lambda: f(*a)


def _seg(name, f):
    del name
    f()


def _region(name, f):
    del name
    f()


def kernel(xa, ka, va, wqa, woa, xb, kb, vb, wqb, wob, out_hbm,
           xt_buf, x_buf, k_buf, v_buf, wq_buf, wo_buf, q_buf, acc, ostage, dummy,
           sems, psem, osem):

    def col0(gg):
        return gg * HW if isinstance(gg, int) else pl.multiple_of(gg * HW, HW)

    def cp_wq(wq_h, gg, slot):
        return pltpu.make_async_copy(wq_h.at[:, pl.ds(col0(gg), HW)], wq_buf.at[slot], sems.at[slot, 0])

    def cp_k(k_h, gg, slot):
        return pltpu.make_async_copy(k_h.at[:, pl.ds(gg * G, G)], k_buf.at[slot], sems.at[slot, 1])

    def cp_v(v_h, gg, slot):
        return pltpu.make_async_copy(v_h.at[:, pl.ds(gg * G, G)], v_buf.at[slot], sems.at[slot, 2])

    def cp_wo(wo_h, gg, slot):
        return pltpu.make_async_copy(wo_h.at[:, pl.ds(col0(gg), HW)], wo_buf.at[slot], sems.at[slot, 3])

    def start_group_dyn(j, slot):
        @pl.when(j < NSTEP_B)
        def _():
            cp_k(ka, j, slot).start()
            cp_v(va, j, slot).start()
            cp_wo(woa, j, slot).start()

        @pl.when(jnp.logical_and(j >= NSTEP_B, j < NSTEP))
        def _():
            cp_k(kb, j - NSTEP_B, slot).start()
            cp_v(vb, j - NSTEP_B, slot).start()
            cp_wo(wob, j - NSTEP_B, slot).start()

        @pl.when(j + 1 < NSTEP_B)
        def _():
            cp_wq(wqa, j + 1, slot).start()

        @pl.when(jnp.logical_and(j + 1 >= NSTEP_B, j + 1 < NSTEP))
        def _():
            cp_wq(wqb, j + 1 - NSTEP_B, slot).start()

    def cp_x(x_h, s, b0, nb, sem):
        return pltpu.make_async_copy(x_h.at[pl.ds(b0, nb)], xt_buf.at[s, pl.ds(b0, nb)], psem.at[sem])

    def cp_kv0(b0, nb, sem):
        return (pltpu.make_async_copy(ka.at[pl.ds(b0, nb), pl.ds(0, G)], k_buf.at[0, pl.ds(b0, nb)], psem.at[sem]),
                pltpu.make_async_copy(va.at[pl.ds(b0, nb), pl.ds(0, G)], v_buf.at[0, pl.ds(b0, nb)], psem.at[sem + 1]))

    def out_copy(b, c0, n, sem):
        return pltpu.make_async_copy(ostage.at[b, :, pl.ds(c0, n)], out_hbm.at[b, :, pl.ds(c0, n)], osem.at[sem])

    def xpose_x(s, b):
        x_buf[s, pl.ds(b * SQ, SQ), :] = xt_buf[s, b].T

    def make_jobs(q_wslot, q_s, q_dst, kv_slot, s, q_src):
        r0 = s * D if isinstance(s, int) else pl.multiple_of(s * D, 8)
        svals, ovals = {}, {}

        def jobQ(b):
            x = x_buf[q_s, pl.ds(b * SQ, SQ), :]
            q = lax.dot_general(x, wq_buf[q_wslot], NN, preferred_element_type=F32)
            q = (q * SCALE).astype(BF16)
            for h in range(G * REP):
                q_buf[q_dst, h // REP, b, pl.ds((h % REP) * SQ, SQ), :] = q[:, h * DH:(h + 1) * DH]

        def jobS(b):
            for j in range(G):
                sc = lax.dot_general(q_buf[q_src, j, b], k_buf[kv_slot, b, j], NT, preferred_element_type=F32)
                m = jnp.max(sc, axis=-1, keepdims=True)
                p = jnp.exp2(sc - m)
                l = jnp.sum(p, axis=-1, keepdims=True)
                svals[b, j] = (p.astype(BF16), l)

        def jobP(b):
            for j in range(G):
                p, l = svals.pop((b, j))
                o = lax.dot_general(p, v_buf[kv_slot, b, j], NN, preferred_element_type=F32)
                inv = pltpu.reciprocal(l, approx=True)
                inv = inv * (2.0 - l * inv)
                ovals[b, j] = (o * inv).astype(BF16)

        def jobO(b):
            parts = []
            for j in range(G):
                o = ovals.pop((b, j))
                parts += [o[:SQ], o[SQ:]]
            ob = jnp.concatenate(parts, axis=1)
            r = lax.dot_general(wo_buf[kv_slot], ob, NT, preferred_element_type=F32)
            acc[pl.ds(r0, D), pl.ds(b * SQ, SQ)] += r

        return dict(Q=jobQ, S=jobS, P=jobP, O=jobO)

    def run_jobs(jobs, order, hooks):
        segs = []
        for name in order:
            if name in hooks or not segs:
                segs.append([])
            segs[-1].append(name)
        for seg in segs:
            def run_seg(seg=seg):
                if seg[0] in hooks:
                    hooks[seg[0]]()
                for name in seg:
                    jobs[name[0]](int(name[1:]))
            _seg(seg[0], run_seg)

    q_order = [f"Q{b}" for b in range(B)]
    spo_order = []
    for b in range(B):
        spo_order += [f"S{b}", f"P{b}"]
    spo_order += [f"O{b}" for b in range(B)]

    x01, x27, xbc = cp_x(xa, 0, 0, 2, 0), cp_x(xa, 0, 2, 6, 1), cp_x(xb, 1, 0, B, 6)
    kva, kvb = cp_kv0(0, 4, 2), cp_kv0(4, 4, 4)

    def p0():
        x01.start()
        cp_wq(wqa, 0, NS).start()
        x27.start()
        acc[...] = jnp.zeros(acc.shape, F32)

    _region("p0", p0)

    def h_q0():
        cp_wq(wqa, 0, NS).wait()
        x01.wait()
        cp_wq(wqa, 1, 0).start()
        xpose_x(0, 0)
        xpose_x(0, 1)

    def h_q2():
        x27.wait()
        kva[0].start()
        kva[1].start()
        for b in range(2, B):
            xpose_x(0, b)

    _region("q0", lambda: run_jobs(make_jobs(NS, 0, 0, 0, 0, 0), q_order, {"Q0": h_q0, "Q2": h_q2}))

    def h_q1():
        cp_wq(wqa, 1, 0).wait()
        kvb[0].start()
        kvb[1].start()
        cp_wo(woa, 0, 0).start()

    _region("q1", lambda: run_jobs(make_jobs(0, 0, 1, 0, 0, 0), q_order, {"Q0": h_q1}))

    def h_s0():
        kva[0].wait()
        kva[1].wait()
        cp_k(ka, 1, 1).start()
        cp_v(va, 1, 1).start()
        cp_wo(woa, 1, 1).start()
        cp_wq(wqa, 2, 1).start()

    def h_s4():
        kvb[0].wait()
        kvb[1].wait()
        cp_wo(woa, 0, 0).wait()
        cp_k(ka, 2, 2).start()
        cp_v(va, 2, 2).start()
        cp_wo(woa, 2, 2).start()
        cp_wq(wqa, 3, 2).start()
        xbc.start()

    _region("s0", lambda: run_jobs(make_jobs(0, 0, 0, 0, 0, 0), spo_order, {"S0": h_s0, "S4": h_s4}))

    def body(i, slot):
        s = lax.shift_right_logical(i, 3)
        qs = lax.shift_right_logical(i + 1, 3)
        qsrc = lax.bitwise_and(i, 1)
        pslot = jnp.where(slot == 0, NS - 1, slot - 1)

        @pl.when(i == 3)
        def _():
            xbc.wait()

        cp_k(ka, 0, slot).wait()
        cp_v(va, 0, slot).wait()
        cp_wo(woa, 0, slot).wait()
        cp_wq(wqa, 0, slot).wait()
        jobs = make_jobs(slot, qs, 1 - qsrc, slot, s, qsrc)

        def xb_loop():
            src = jnp.where(i >= 3, 1, 0)
            b0 = pl.multiple_of(lax.bitwise_and(2 * i + 2, B - 1), 2)
            for t in range(2):
                x_buf[1, pl.ds(pl.multiple_of((b0 + t) * SQ, SQ), SQ), :] = xt_buf[src, b0 + t].T

        hk = {HK1: lambda: start_group_dyn(i + 2, pslot), HK2: xb_loop}
        run_jobs(jobs, (q_order + spo_order) if ORD == "QF" else (spo_order + q_order), hk)
        return jnp.where(slot == NS - 1, 0, slot + 1)

    _region("loop", lambda: lax.fori_loop(1, NSTEP - 1, body, jnp.int32(1)))

    def fin(b, c0, n, sem):
        ostage[b, :, c0:c0 + n] = acc[c0:c0 + n, pl.ds(b * SQ, SQ)].T.astype(BF16)
        out_copy(b, c0, n, sem).start()

    def last():
        i = NSTEP - 1
        slot = i % NS
        cp_k(ka, 0, slot).wait()
        cp_v(va, 0, slot).wait()
        cp_wo(woa, 0, slot).wait()
        dcp = pltpu.make_async_copy(xa.at[0, pl.ds(0, 16)], dummy, psem.at[7])
        dcp.start()
        order = ["S0", "P0"]
        for b in range(1, B):
            order += [f"S{b}", f"O{b - 1}", f"P{b}"]
        order += [f"O{B - 1}"]
        hooks = {}
        def fin_a():
            for b in range(B):
                fin(b, 0, 512, b)
        hooks["S0"] = fin_a
        for b in range(B - 1):
            nxt = f"P{b + 1}"
            f = _bind(fin, b, 512, 640, B + b)
            if b == KSPLIT:
                hooks[f"S{b + 1}"] = dcp.wait
            hooks[nxt] = f
        run_jobs(make_jobs(0, 1, 0, slot, 1, i % 2), order, hooks)
        fin(B - 1, 512, 640, 2 * B - 1)
        for b in range(B):
            out_copy(b, 0, 512, b).wait()
            out_copy(b, 512, 640, B + b).wait()

    _region("last", last)


@jax.jit
def pallas_concat_heads__gqa_block_cached__gqa_block_cached__near_ridge_kernel(A_x, A_k_cache, A_v_cache, A_wq, A_wo, B_x, B_k_cache, B_v_cache, B_wq, B_wo):
    hbm = pl.BlockSpec(memory_space=pltpu.HBM)
    return pl.pallas_call(
        kernel,
        grid=(1,),
        in_specs=[hbm] * 10,
        out_specs=hbm,
        out_shape=jax.ShapeDtypeStruct((B, SQ, 2 * D), BF16),
        scratch_shapes=[
            pltpu.VMEM((2, B, D, SQ), BF16),
            pltpu.VMEM((2, B * SQ, D), BF16),
            pltpu.VMEM((NS, B, G, SK, DH), BF16),
            pltpu.VMEM((NS, B, G, SK, DH), BF16),
            pltpu.VMEM((NS + 1, D, HW), BF16),
            pltpu.VMEM((NS, D, HW), BF16),
            pltpu.VMEM((2, G, B, REP * SQ, DH), BF16),
            pltpu.VMEM((2 * D, B * SQ), F32),
            pltpu.VMEM((B, SQ, 2 * D), BF16),
            pltpu.VMEM((16, SQ), BF16),
            pltpu.SemaphoreType.DMA((NS + 1, 4)),
            pltpu.SemaphoreType.DMA((8,)),
            pltpu.SemaphoreType.DMA((2 * B,)),
        ],
        compiler_params=pltpu.CompilerParams(
            vmem_limit_bytes=100 * 1024 * 1024, disable_bounds_checks=True),
    )(A_x.transpose(0, 2, 1), A_k_cache, A_v_cache, A_wq, A_wo.T,
      B_x.transpose(0, 2, 1), B_k_cache, B_v_cache, B_wq, B_wo.T)
```

```python
import jax
import jax.numpy as jnp
from jax import lax
import jax.experimental.pallas as pl
import jax.experimental.pallas.tpu as pltpu

B, SQ, D = 8, 128, 576
HKV, SK, DH = 16, 512, 128
REP = 2
G = 2
NSTEP_B = HKV // G
NSTEP = 2 * NSTEP_B
HW = G * REP * DH
NS = 3
NT = (((1,), (1,)), ((), ()))
NN = (((1,), (0,)), ((), ()))
SCALE = float(DH ** -0.5 * 1.4426950408889634)
F32, BF16 = jnp.float32, jnp.bfloat16

KSPLIT = 6


def _bind(f, *a):
    return lambda: f(*a)


def kernel(xa, ka, va, wqa, woa, xb, kb, vb, wqb, wob, out_hbm,
           xt_buf, x_buf, k_buf, v_buf, wq_buf, wo_buf, q_buf, acc, ostage, dummy,
           sems, psem, osem):

    def col0(gg):
        return gg * HW if isinstance(gg, int) else pl.multiple_of(gg * HW, HW)

    def cp_wq(wq_h, gg, slot):
        return pltpu.make_async_copy(wq_h.at[:, pl.ds(col0(gg), HW)], wq_buf.at[slot], sems.at[slot, 0])

    def cp_k(k_h, gg, slot):
        return pltpu.make_async_copy(k_h.at[:, pl.ds(gg * G, G)], k_buf.at[slot], sems.at[slot, 1])

    def cp_v(v_h, gg, slot):
        return pltpu.make_async_copy(v_h.at[:, pl.ds(gg * G, G)], v_buf.at[slot], sems.at[slot, 2])

    def cp_wo(wo_h, gg, slot):
        return pltpu.make_async_copy(wo_h.at[:, pl.ds(col0(gg), HW)], wo_buf.at[slot], sems.at[slot, 3])

    def start_group_dyn(j, slot):
        @pl.when(j < NSTEP_B)
        def _():
            cp_k(ka, j, slot).start()
            cp_v(va, j, slot).start()
            cp_wo(woa, j, slot).start()

        @pl.when(jnp.logical_and(j >= NSTEP_B, j < NSTEP))
        def _():
            cp_k(kb, j - NSTEP_B, slot).start()
            cp_v(vb, j - NSTEP_B, slot).start()
            cp_wo(wob, j - NSTEP_B, slot).start()

        @pl.when(j + 1 < NSTEP_B)
        def _():
            cp_wq(wqa, j + 1, slot).start()

        @pl.when(jnp.logical_and(j + 1 >= NSTEP_B, j + 1 < NSTEP))
        def _():
            cp_wq(wqb, j + 1 - NSTEP_B, slot).start()

    def cp_x(x_h, s, b0, nb, sem):
        return pltpu.make_async_copy(x_h.at[pl.ds(b0, nb)], xt_buf.at[s, pl.ds(b0, nb)], psem.at[sem])

    def cp_kv0(b0, nb, sem):
        return (pltpu.make_async_copy(ka.at[pl.ds(b0, nb), pl.ds(0, G)], k_buf.at[0, pl.ds(b0, nb)], psem.at[sem]),
                pltpu.make_async_copy(va.at[pl.ds(b0, nb), pl.ds(0, G)], v_buf.at[0, pl.ds(b0, nb)], psem.at[sem + 1]))

    def out_copy(b, c0, n, sem):
        return pltpu.make_async_copy(ostage.at[b, :, pl.ds(c0, n)], out_hbm.at[b, :, pl.ds(c0, n)], osem.at[sem])

    def xpose_x(s, b):
        x_buf[s, pl.ds(b * SQ, SQ), :] = xt_buf[s, b].T

    def make_jobs(q_wslot, q_s, q_dst, kv_slot, s, q_src):
        r0 = s * D if isinstance(s, int) else pl.multiple_of(s * D, 8)
        svals, ovals = {}, {}

        def jobQ(b):
            x = x_buf[q_s, pl.ds(b * SQ, SQ), :]
            q = lax.dot_general(x, wq_buf[q_wslot], NN, preferred_element_type=F32)
            q = (q * SCALE).astype(BF16)
            for h in range(G * REP):
                q_buf[q_dst, h // REP, b, pl.ds((h % REP) * SQ, SQ), :] = q[:, h * DH:(h + 1) * DH]

        def jobS(b):
            for j in range(G):
                sc = lax.dot_general(q_buf[q_src, j, b], k_buf[kv_slot, b, j], NT, preferred_element_type=F32)
                m = jnp.max(sc, axis=-1, keepdims=True)
                p = jnp.exp2(sc - m)
                l = jnp.sum(p, axis=-1, keepdims=True)
                svals[b, j] = (p.astype(BF16), l)

        def jobP(b):
            for j in range(G):
                p, l = svals.pop((b, j))
                o = lax.dot_general(p, v_buf[kv_slot, b, j], NN, preferred_element_type=F32)
                inv = pltpu.reciprocal(l, approx=True)
                inv = inv * (2.0 - l * inv)
                ovals[b, j] = (o * inv).astype(BF16)

        def jobO(b):
            parts = []
            for j in range(G):
                o = ovals.pop((b, j))
                parts += [o[:SQ], o[SQ:]]
            ob = jnp.concatenate(parts, axis=1)
            r = lax.dot_general(wo_buf[kv_slot], ob, NT, preferred_element_type=F32)
            acc[pl.ds(r0, D), pl.ds(b * SQ, SQ)] += r

        return dict(Q=jobQ, S=jobS, P=jobP, O=jobO)

    def run_jobs(jobs, order, hooks):
        for name in order:
            if name in hooks:
                hooks[name]()
            jobs[name[0]](int(name[1:]))

    q_order = [f"Q{b}" for b in range(B)]
    spo_order = []
    for b in range(B):
        spo_order += [f"S{b}", f"P{b}"]
    spo_order += [f"O{b}" for b in range(B)]

    x01, x27, xbc = cp_x(xa, 0, 0, 2, 0), cp_x(xa, 0, 2, 6, 1), cp_x(xb, 1, 0, B, 6)
    kva, kvb = cp_kv0(0, 4, 2), cp_kv0(4, 4, 4)

    def p0():
        x01.start()
        cp_wq(wqa, 0, NS).start()
        x27.start()
        acc[...] = jnp.zeros(acc.shape, F32)

    p0()

    def h_q0():
        cp_wq(wqa, 0, NS).wait()
        x01.wait()
        cp_wq(wqa, 1, 0).start()
        xpose_x(0, 0)
        xpose_x(0, 1)

    def h_q2():
        x27.wait()
        kva[0].start()
        kva[1].start()
        for b in range(2, B):
            xpose_x(0, b)

    run_jobs(make_jobs(NS, 0, 0, 0, 0, 0), q_order, {"Q0": h_q0, "Q2": h_q2})

    def h_q1():
        cp_wq(wqa, 1, 0).wait()
        kvb[0].start()
        kvb[1].start()
        cp_wo(woa, 0, 0).start()

    run_jobs(make_jobs(0, 0, 1, 0, 0, 0), q_order, {"Q0": h_q1})

    def h_s0():
        kva[0].wait()
        kva[1].wait()
        cp_k(ka, 1, 1).start()
        cp_v(va, 1, 1).start()
        cp_wo(woa, 1, 1).start()
        cp_wq(wqa, 2, 1).start()

    def h_s4():
        kvb[0].wait()
        kvb[1].wait()
        cp_wo(woa, 0, 0).wait()
        cp_k(ka, 2, 2).start()
        cp_v(va, 2, 2).start()
        cp_wo(woa, 2, 2).start()
        cp_wq(wqa, 3, 2).start()
        xbc.start()

    run_jobs(make_jobs(0, 0, 0, 0, 0, 0), spo_order, {"S0": h_s0, "S4": h_s4})

    def body(i, slot):
        s = lax.shift_right_logical(i, 3)
        qs = lax.shift_right_logical(i + 1, 3)
        qsrc = lax.bitwise_and(i, 1)
        pslot = jnp.where(slot == 0, NS - 1, slot - 1)

        @pl.when(i == 3)
        def _():
            xbc.wait()

        cp_k(ka, 0, slot).wait()
        cp_v(va, 0, slot).wait()
        cp_wo(woa, 0, slot).wait()
        cp_wq(wqa, 0, slot).wait()
        jobs = make_jobs(slot, qs, 1 - qsrc, slot, s, qsrc)

        def xb_loop():
            src = jnp.where(i >= 3, 1, 0)
            b0 = pl.multiple_of(lax.bitwise_and(2 * i + 2, B - 1), 2)
            for t in range(2):
                x_buf[1, pl.ds(pl.multiple_of((b0 + t) * SQ, SQ), SQ), :] = xt_buf[src, b0 + t].T

        hk = {"Q1": lambda: start_group_dyn(i + 2, pslot), "S2": xb_loop}
        run_jobs(jobs, q_order + spo_order, hk)
        return jnp.where(slot == NS - 1, 0, slot + 1)

    lax.fori_loop(1, NSTEP - 1, body, jnp.int32(1))

    def fin(b, c0, n, sem):
        ostage[b, :, c0:c0 + n] = acc[c0:c0 + n, pl.ds(b * SQ, SQ)].T.astype(BF16)
        out_copy(b, c0, n, sem).start()

    def last():
        i = NSTEP - 1
        slot = i % NS
        cp_k(ka, 0, slot).wait()
        cp_v(va, 0, slot).wait()
        cp_wo(woa, 0, slot).wait()
        dcp = pltpu.make_async_copy(xa.at[0, pl.ds(0, 16)], dummy, psem.at[7])
        dcp.start()
        order = ["S0", "P0"]
        for b in range(1, B):
            order += [f"S{b}", f"O{b - 1}", f"P{b}"]
        order += [f"O{B - 1}"]
        hooks = {}
        def fin_a():
            for b in range(B):
                fin(b, 0, 512, b)
        hooks["S0"] = fin_a
        for b in range(B - 1):
            nxt = f"P{b + 1}"
            f = _bind(fin, b, 512, 640, B + b)
            if b == KSPLIT:
                hooks[f"S{b + 1}"] = dcp.wait
            hooks[nxt] = f
        run_jobs(make_jobs(0, 1, 0, slot, 1, i % 2), order, hooks)
        fin(B - 1, 512, 640, 2 * B - 1)
        for b in range(B):
            out_copy(b, 0, 512, b).wait()
            out_copy(b, 512, 640, B + b).wait()

    last()


@jax.jit
def pallas_concat_heads__gqa_block_cached__gqa_block_cached__near_ridge_kernel(A_x, A_k_cache, A_v_cache, A_wq, A_wo, B_x, B_k_cache, B_v_cache, B_wq, B_wo):
    hbm = pl.BlockSpec(memory_space=pltpu.HBM)
    return pl.pallas_call(
        kernel,
        grid=(1,),
        in_specs=[hbm] * 10,
        out_specs=hbm,
        out_shape=jax.ShapeDtypeStruct((B, SQ, 2 * D), BF16),
        scratch_shapes=[
            pltpu.VMEM((2, B, D, SQ), BF16),
            pltpu.VMEM((2, B * SQ, D), BF16),
            pltpu.VMEM((NS, B, G, SK, DH), BF16),
            pltpu.VMEM((NS, B, G, SK, DH), BF16),
            pltpu.VMEM((NS + 1, D, HW), BF16),
            pltpu.VMEM((NS, D, HW), BF16),
            pltpu.VMEM((2, G, B, REP * SQ, DH), BF16),
            pltpu.VMEM((2 * D, B * SQ), F32),
            pltpu.VMEM((B, SQ, 2 * D), BF16),
            pltpu.VMEM((16, SQ), BF16),
            pltpu.SemaphoreType.DMA((NS + 1, 4)),
            pltpu.SemaphoreType.DMA((8,)),
            pltpu.SemaphoreType.DMA((2 * B,)),
        ],
        compiler_params=pltpu.CompilerParams(
            vmem_limit_bytes=100 * 1024 * 1024, disable_bounds_checks=True),
    )(A_x.transpose(0, 2, 1), A_k_cache, A_v_cache, A_wq, A_wo.T,
      B_x.transpose(0, 2, 1), B_k_cache, B_v_cache, B_wq, B_wo.T)
```
